```python
import os as _os
_os.environ.setdefault("JAX_PLATFORMS", "cpu")
import jax
import jax.numpy as jnp

def _softmax(x, axis=-1):
    return jax.nn.softmax(x, axis=axis)
def _gelu(x):
    return jax.nn.gelu(x, approximate=True)
def _silu(x):
    return jax.nn.silu(x)
def _sigmoid(x):
    return jax.nn.sigmoid(x)
def _layernorm(x, axis=-1, eps=1e-5):
    m = jnp.mean(x, axis=axis, keepdims=True)
    v = jnp.var(x, axis=axis, keepdims=True)
    return (x - m) / jnp.sqrt(v + eps)
def _scatter_add(tgt, idx, src, axis=0):
    return tgt.at[idx].add(src)
def _segment_sum(src, seg, n):
    return jax.ops.segment_sum(src, seg, n)
class _Rng:
    def __init__(self, key):
        self._k = key
    def _next(self):
        self._k, sub = jax.random.split(self._k)
        return sub
    def normal(self, shape):
        return jax.random.normal(self._next(), shape, dtype=jnp.bfloat16)
    def randint(self, lo, hi, shape):
        return jax.random.randint(self._next(), shape, lo, hi, dtype=jnp.int32)
    def uniform(self, shape, lo=0.0, hi=1.0):
        return jax.random.uniform(self._next(), shape, jnp.bfloat16, lo, hi)
    def permutation(self, n):
        return jax.random.permutation(self._next(), n)


kernel_name = 'parallel_sum__ssm_conv_s5__geglu_ffn__prompt'

def setup_inputs():
    _rng = _Rng(jax.random.key(int.from_bytes(__import__("os").urandom(4), "little")))
    _w = (lambda a: (lambda t: t.astype(jnp.bfloat16) if jnp.issubdtype(t.dtype, jnp.floating) else t)(jnp.asarray(a)))
    def _A_setup():
        B, S, D = 1, 2048, 512
        P = D
        Lambda_re = -0.5 * jnp.exp((lambda *s: _rng.normal(s) * 0.8)(P))
        Lambda_im = (lambda *s: _rng.normal(s) * 0.8)(P) * 1.0
        B_re = (lambda *s: _rng.normal(s) * 0.8)(P, D) * (D ** -0.5)
        B_im = (lambda *s: _rng.normal(s) * 0.8)(P, D) * (D ** -0.5)
        C_re = (lambda *s: _rng.normal(s) * 0.8)(D, P) * (P ** -0.5)
        C_im = (lambda *s: _rng.normal(s) * 0.8)(D, P) * (P ** -0.5)
        log_dt = (lambda *s: _rng.normal(s) * 0.8)(P) * 0.3 - 2.0
        Dskip = (lambda *s: _rng.normal(s) * 0.8)(D)
        return {
            "x": _w((lambda *s: _rng.normal(s) * 0.05)(B, S, D)),
            "Lambda_re": _w(Lambda_re),
            "Lambda_im": _w(Lambda_im),
            "B_re": _w(B_re),
            "B_im": _w(B_im),
            "C_re": _w(C_re),
            "C_im": _w(C_im),
            "log_dt": _w(log_dt),
            "Dskip": _w(Dskip),
        }
    _A_in = _A_setup()

    def _B_setup():
        B, S, D, F = 1, 2048, 512, 1376
        return {
            "x": _w((lambda *s: _rng.normal(s) * 0.05)(B, S, D)),
            "w_gate": _w((lambda *s: _rng.normal(s) * 0.05)(D, F)),
            "w_up": _w((lambda *s: _rng.normal(s) * 0.05)(D, F)),
            "w_down": _w((lambda *s: _rng.normal(s) * 0.05)(F, D)),
        }
    _B_in = _B_setup()

    return {
        "A_x": _A_in["x"],
        "A_Lambda_re": _A_in["Lambda_re"],
        "A_Lambda_im": _A_in["Lambda_im"],
        "A_B_re": _A_in["B_re"],
        "A_B_im": _A_in["B_im"],
        "A_C_re": _A_in["C_re"],
        "A_C_im": _A_in["C_im"],
        "A_log_dt": _A_in["log_dt"],
        "A_Dskip": _A_in["Dskip"],
        "B_x": _B_in["x"],
        "B_w_gate": _B_in["w_gate"],
        "B_w_up": _B_in["w_up"],
        "B_w_down": _B_in["w_down"],
    }

def reference(A_x, A_Lambda_re, A_Lambda_im, A_B_re, A_B_im, A_C_re, A_C_im, A_log_dt, A_Dskip, B_x, B_w_gate, B_w_up, B_w_down):
    def _A_ref(x, Lambda_re, Lambda_im, B_re, B_im, C_re, C_im, log_dt, Dskip):
        Bsz, L, H = x.shape
        Lam = Lambda_re + 1j * Lambda_im
        Bmat = B_re + 1j * B_im
        Cmat = C_re + 1j * C_im
        dt = jnp.exp(log_dt)
        Lam_bar = jnp.exp(dt * Lam)
        B_bar = ((Lam_bar - 1.0) / Lam)[:, None] * Bmat
        Bu = jnp.einsum("bld,pd->blp", x + 0j, B_bar)
        h = jnp.zeros_like(Bu[:, 0, :])
        hs = []
        for t in range(L):
            h = Lam_bar[None, :] * h + Bu[:, t, :]
            hs.append(h)
        hseq = jnp.stack(hs, 1)
        y = 2.0 * jnp.einsum("blp,dp->bld", hseq, Cmat).real + x * Dskip[None, None, :]
        return y

    def _B_ref(x, w_gate, w_up, w_down):
        return (_gelu(x @ w_gate) * (x @ w_up)) @ w_down

    x = A_x
    xn = _layernorm(x, axis=-1)
    return x + _A_ref(xn, A_Lambda_re, A_Lambda_im, A_B_re, A_B_im, A_C_re, A_C_im, A_log_dt, A_Dskip) + _B_ref(xn, B_w_gate, B_w_up, B_w_down)
```

```python
import functools
import jax, jax.numpy as jnp, numpy as np
from jax import lax
import jax.experimental.pallas as pl
import jax.experimental.pallas.tpu as pltpu

L, D, P, F = 2048, 512, 512, 1376
BF = jnp.bfloat16
F32 = jnp.float32
U32 = jnp.uint32
C0 = float(np.sqrt(2.0 / np.pi))
C1 = float(np.sqrt(2.0 / np.pi) * 0.044715)
NC = 4

def cmul(ar, ai, br, bi):
    return ar * br - ai * bi, ar * bi + ai * br

def nt_dot(a, b):
    return lax.dot_general(a, b, (((1,), (1,)), ((), ())), preferred_element_type=F32)

def nn_dot(a, b):
    return jnp.dot(a, b, preferred_element_type=F32)

def to_u32(v):
    return pltpu.bitcast(v, U32)

def to_bf(v):
    return pltpu.bitcast(v, BF)

class Bg:
    def __init__(self):
        self.q = []
    def add(self, gen):
        self.q.append(gen)
    def step(self, n=1):
        while n > 0 and self.q:
            try:
                next(self.q[0]); n -= 1
            except StopIteration:
                self.q.pop(0)
    def drain(self):
        self.step(1 << 30)

def build(R=256, S=8, FC=128, BC=128, vmem=100, nodma=False, flags=None, pg=4, frac=0.9, lnp=1,
          xg=(256, 256, 256, 1280), odma=1, dcpos=8, cpieces=8):
    NR = L // R
    TS = 8 * S
    fch = [(f0, min(FC, F - f0)) for f0 in range(0, F, FC)]
    bch = [(b0, BC) for b0 in range(0, P, BC)]
    xoff = np.cumsum((0,) + tuple(xg))
    assert xoff[-1] == L
    NXG = len(xg)

    def kernel(x_hbm, lre_hbm, lim_hbm, ldt_hbm, bre_hbm, bim_hbm, cre_hbm, cim_hbm, dsk_hbm,
               wg_hbm, wu_hbm, wd_hbm, o_hbm, *scr):
        scr = list(scr)
        xbufs = [scr.pop(0) for _ in range(NXG)]
        obufs = [scr.pop(0) for _ in range(NR)]
        (v_lre, v_lim, v_ldt, v_dsk, bre, bim, cre, cim, cpr, cpi, wg, wu, wd,
         xp, res, ubuf, hbuf, act, tab, sem) = scr
        class _Nop:
            def start(self): pass
            def wait(self): pass
        def mk(src, dst, sem):
            return _Nop() if nodma else pltpu.make_async_copy(src, dst, sem)
        def cg(src, dst, s, r0=None, r1=None):
            if r0 is None:
                return [mk(src.at[:, pl.ds(c * 128, 128)], dst.at[c], sem.at[s]) for c in range(NC)]
            return [mk(src.at[pl.ds(r0, r1 - r0), pl.ds(c * 128, 128)], dst.at[c], sem.at[s]) for c in range(NC)]
        grp = {}
        xg_ = lambda i, s: cg(x_hbm, xbufs[i], s, int(xoff[i]), int(xoff[i + 1]))
        grp["x0"] = xg_(0, 0)
        grp["bre"] = cg(bre_hbm, bre, 1)
        grp["x1"] = xg_(1, 2)
        grp["bim"] = cg(bim_hbm, bim, 3)
        grp["x2"] = xg_(2, 3) + [mk(s, d, sem.at[3]) for s, d in ((lre_hbm, v_lre), (lim_hbm, v_lim), (ldt_hbm, v_ldt), (dsk_hbm, v_dsk))]
        grp["x3"] = xg_(3, 4)
        grp["gu"] = cg(wg_hbm, wg, 5) + cg(wu_hbm, wu, 5)
        grp["dc"] = [mk(cre_hbm, cre, sem.at[6]), mk(cim_hbm, cim, sem.at[6])] + cg(wd_hbm, wd, 6)
        for k in grp:
            for c in grp[k]:
                c.start()
        def wait(*ks):
            for k in ks:
                for c in grp[k]:
                    c.wait()

        def ldw(ref, r0, rn, cs=(0, 1, 2, 3)):
            u = ref.bitcast(U32)
            return to_bf(jnp.concatenate([u[c, r0 // 2:(r0 + rn) // 2, :] for c in cs], axis=1))
        def ld(ref, r0, rn, c0=None, cn=None):
            if c0 is None:
                return to_bf(ref[r0 // 2:(r0 + rn) // 2, :])
            return to_bf(ref[r0 // 2:(r0 + rn) // 2, c0:c0 + cn])

        def ln_pieces(t_lo, t_hi):
            for t0 in range(t_lo, t_hi, TS):
                gi = int(np.searchsorted(xoff, t0, side="right") - 1)
                xu = xbufs[gi].bitcast(U32)
                q0 = (t0 - int(xoff[gi])) // 2
                los, his = [], []
                for ip in range(S // 2):
                    w = jnp.concatenate([xu[c, pl.ds(q0 + ip, 8, stride=S // 2), :] for c in range(NC)], axis=1)
                    los.append(pltpu.bitcast(w << 16, F32))
                    his.append(pltpu.bitcast(w & jnp.uint32(0xFFFF0000), F32))
                rows = []
                for i in range(S):
                    rows.append(los[i // 2] if i % 2 == 0 else his[i // 2])
                x = jnp.concatenate(rows, axis=0)
                res[t0:t0 + TS, :] = x
                m = jnp.mean(x, axis=-1, keepdims=True)
                if lnp: yield
                xc = x - m
                v = jnp.mean(xc * xc, axis=-1, keepdims=True)
                if lnp: yield
                xnb = (xc * lax.rsqrt(v + 1e-5)).astype(BF)
                xp[t0 // 2:(t0 + TS) // 2, :] = to_u32(xnb)
                yield

        def bproj(r, part, tick):
            lhs = ld(xp, r * R, R)
            w = (bre, bim)[part]
            for (b0, bn) in bch:
                ubuf[r * R:(r + 1) * R, part * P + b0:part * P + b0 + bn] = nt_dot(lhs, ldw(w, b0, bn))
                tick()

        def prep_tables():
            lre = v_lre[...].astype(F32).reshape(1, P)
            lim = v_lim[...].astype(F32).reshape(1, P)
            dt = jnp.exp(v_ldt[...].astype(F32).reshape(1, P)).astype(BF).astype(F32)
            zr, zi = dt * lre, dt * lim
            yield
            mag = jnp.exp(zr)
            ar = mag * jnp.cos(zi)
            yield
            ai = mag * jnp.sin(zi)
            yield
            nr, ni = ar - 1.0, ai
            den = lre * lre + lim * lim
            sr = (nr * lre + ni * lim) / den
            si = (ni * lre - nr * lim) / den
            sub = lax.broadcasted_iota(jnp.int32, (8, P), 0)
            tab[0] = jnp.broadcast_to(ar, (8, P))
            tab[1] = jnp.broadcast_to(ai, (8, P))
            tab[8] = jnp.broadcast_to(2.0 * sr, (8, P))
            tab[9] = jnp.broadcast_to(2.0 * si, (8, P))
            yield
            pr, pi_ = ar, ai
            n = 1
            while n < S:
                pr, pi_ = cmul(pr, pi_, pr, pi_)
                n *= 2
            for k, d in enumerate((1, 2, 4)):
                tab[2 + 2 * k] = jnp.where(sub >= d, jnp.broadcast_to(pr, (8, P)), 0.0)
                tab[3 + 2 * k] = jnp.where(sub >= d, jnp.broadcast_to(pi_, (8, P)), 0.0)
                pr, pi_ = cmul(pr, pi_, pr, pi_)
            yield

        def prep_c(nparts):
            for part in range(nparts):
                r0, r1 = part * D // nparts, (part + 1) * D // nparts
                sr2, si2 = tab[8][0:1, :], tab[9][0:1, :]
                c_re = cre[r0:r1, :].astype(F32)
                c_im = cim[r0:r1, :].astype(F32)
                cpr[r0 // 2:r1 // 2, :] = to_u32((c_re * sr2 - c_im * si2).astype(BF))
                cpi[r0 // 2:r1 // 2, :] = to_u32((-(c_re * si2) - c_im * sr2).astype(BF))
                yield

        def gu(r, tick):
            lhs = ld(xp, r * R, R)
            for (f0, fn) in fch:
                g = nt_dot(lhs, ldw(wg, f0, fn))
                tick()
                u = nt_dot(lhs, ldw(wu, f0, fn))
                t = jnp.tanh(g * (C0 + C1 * (g * g)))
                act[r * R // 2:(r + 1) * R // 2, f0:f0 + fn] = to_u32(((g * u) * (0.5 + 0.5 * t)).astype(BF))
                tick()

        def scan_pieces():
            sub = lax.broadcasted_iota(jnp.int32, (8, P), 0)
            cr = ci = jnp.zeros((8, P), F32)
            for base in range(0, L, TS):
                ar, ai = tab[0], tab[1]
                fr = ubuf[base:base + 8, 0:P]
                fi = ubuf[base:base + 8, P:2 * P]
                for i in range(1, S):
                    ur = ubuf[base + 8 * i:base + 8 * i + 8, 0:P]
                    ui = ubuf[base + 8 * i:base + 8 * i + 8, P:2 * P]
                    fr, fi = ar * fr - ai * fi + ur, ar * fi + ai * fr + ui
                    if pg and i % pg == pg - 1 and i < S - 1: yield
                yield
                hr = jnp.where(sub == 0, cr, pltpu.roll(fr, 1, 0))
                hi = jnp.where(sub == 0, ci, pltpu.roll(fi, 1, 0))
                for k, d in enumerate((1, 2, 4)):
                    qr, qi = pltpu.roll(hr, d, 0), pltpu.roll(hi, d, 0)
                    tr, ti = tab[2 + 2 * k], tab[3 + 2 * k]
                    hr, hi = hr + (tr * qr - ti * qi), hi + (tr * qi + ti * qr)
                yield
                hs_r, hs_i = [], []
                for i in range(S):
                    ur = ubuf[base + 8 * i:base + 8 * i + 8, 0:P]
                    ui = ubuf[base + 8 * i:base + 8 * i + 8, P:2 * P]
                    hr, hi = ar * hr - ai * hi + ur, ar * hi + ai * hr + ui
                    hs_r.append(hr)
                    hs_i.append(hi)
                    if i % 2 == 1:
                        b2 = (base + 8 * (i - 1)) // 2
                        hbuf[b2:b2 + 8, 0:P] = to_u32(jnp.concatenate(hs_r[-2:], axis=0).astype(BF))
                        hbuf[b2:b2 + 8, P:2 * P] = to_u32(jnp.concatenate(hs_i[-2:], axis=0).astype(BF))
                    if pg and i % pg == pg - 1 and i < S - 1: yield
                cr = jnp.broadcast_to(hr[7:8, :], (8, P))
                ci = jnp.broadcast_to(hi[7:8, :], (8, P))
                yield
        scan_np = (L // TS) * (3 + (2 * (S // pg - 1) if pg else 0))

        osem = sem.at[7]
        ocps = []
        def outp(r, dsk, tick, nsplit=1):
            rows = slice(r * R, (r + 1) * R)
            ys = []
            if r == 0:
                for c in range(NC):
                    ys.append(nn_dot(ld(act, r * R, R), ldw(wd, 0, F, (c,))))
                    tick()
                bg.drain()
            for c in range(NC):
                c0, c1 = c * 128, (c + 1) * 128
                cols = slice(c0, c1)
                y = res[rows, cols] + ld(xp, r * R, R, c0, 128).astype(F32) * dsk[:, cols]
                if r == 0:
                    y = y + ys[c]
                else:
                    y = y + nn_dot(ld(act, r * R, R), ldw(wd, 0, F, (c,)))
                y = y + nt_dot(ld(hbuf, r * R, R, 0, P), ld(cpr, c0, 128))
                y = y + nt_dot(ld(hbuf, r * R, R, P, P), ld(cpi, c0, 128))
                for n in range(R // TS):
                    for i in range(S):
                        r0 = n * TS + i * 8
                        obufs[r][c, pl.ds(n * TS + i, 8, stride=S), :] = y[r0:r0 + 8, :]
                    if (n + 1) % (R // TS // nsplit) == 0:
                        a = (n + 1) * TS - R // nsplit
                        cp = pltpu.make_async_copy(obufs[r].at[c, pl.ds(a, R // nsplit), :],
                                                   o_hbm.at[pl.ds(r * R + a, R // nsplit), pl.ds(c * 128, 128)], osem)
                        cp.start()
                        ocps.append(cp)

        assert R == 256 and tuple(xg[:3]) == (256, 256, 256)
        bg = Bg()
        nop = lambda: None
        wait("x0")
        bg.add(ln_pieces(0, 256)); bg.drain()
        wait("bre")
        bproj(0, 0, nop)
        wait("x1")
        bg.add(ln_pieces(256, 512)); bg.drain()
        bproj(1, 0, nop)
        wait("bim", "x2")
        per = (3 if lnp else 1) * (R // TS)
        bg.add(ln_pieces(512, 768)); bg.add(prep_tables())
        bproj(0, 1, lambda: bg.step(-(-per // len(bch))))
        bproj(1, 1, lambda: bg.step(2))
        bg.drain()
        bproj(2, 0, nop)
        wait("x3")
        bg.add(ln_pieces(768, 2048))
        bproj(2, 1, lambda: bg.step(-(-per // len(bch))))
        for r in range(3, 8):
            for part in range(2):
                bproj(r, part, (lambda: bg.step(-(-per // (2 * len(bch))))) if r < 7 else nop)
        bg.drain()
        wait("gu")
        gen = scan_pieces()
        prog = {"mx": 0, "done": 0}
        total_mx = NR * 2 * len(fch) * frac
        def tick():
            prog["mx"] += 1
            want = min(scan_np, int(np.ceil(scan_np * prog["mx"] / total_mx)))
            while prog["done"] < want:
                next(gen); prog["done"] += 1
        for r in range(NR):
            if r == dcpos:
                wait("dc")
            gu(r, tick)
        for _ in gen:
            pass
        if dcpos >= NR:
            wait("dc")
        bg.add(prep_c(cpieces))
        dsk = v_dsk[...].astype(F32).reshape(1, D)
        for r in range(NR):
            outp(r, dsk, lambda: bg.step(-(-cpieces // NC)), nsplit=(odma if r == NR - 1 else 1))
        for cp in ocps:
            cp.wait()

    def f(A_x, A_Lambda_re, A_Lambda_im, A_B_re, A_B_im, A_C_re, A_C_im, A_log_dt, A_Dskip, B_x, B_w_gate, B_w_up, B_w_down):
        hbm = pl.BlockSpec(memory_space=pltpu.HBM)
        out = pl.pallas_call(
            kernel,
            in_specs=[hbm] * 12,
            out_specs=hbm,
            out_shape=jax.ShapeDtypeStruct((L, D), F32),
            scratch_shapes=[pltpu.VMEM((NC, n, 128), BF) for n in xg] + [pltpu.VMEM((NC, R, 128), F32) for _ in range(NR)] + [
                pltpu.VMEM((P,), BF), pltpu.VMEM((P,), BF), pltpu.VMEM((P,), BF), pltpu.VMEM((D,), BF),
                pltpu.VMEM((NC, P, 128), BF), pltpu.VMEM((NC, P, 128), BF),
                pltpu.VMEM((D, P), BF), pltpu.VMEM((D, P), BF),
                pltpu.VMEM((D // 2, P), U32), pltpu.VMEM((D // 2, P), U32),
                pltpu.VMEM((NC, F, 128), BF), pltpu.VMEM((NC, F, 128), BF), pltpu.VMEM((NC, F, 128), BF),
                pltpu.VMEM((L // 2, D), U32),
                pltpu.VMEM((L, D), F32),
                pltpu.VMEM((L, 2 * P), F32),
                pltpu.VMEM((L // 2, 2 * P), U32),
                pltpu.VMEM((L // 2, F), U32),
                pltpu.VMEM((10, 8, P), F32),
                pltpu.SemaphoreType.DMA((8,)),
            ],
            compiler_params=pltpu.CompilerParams(vmem_limit_bytes=vmem * 2**20, flags=flags),
        )(A_x.reshape(L, D), A_Lambda_re, A_Lambda_im, A_log_dt, A_B_re, A_B_im, A_C_re, A_C_im, A_Dskip,
          B_w_gate.T, B_w_up.T, B_w_down)
        return out.reshape(1, L, D)
    return f


_impl = build()


@jax.jit
def pallas_parallel_sum__ssm_conv_s5__geglu_ffn__prompt_kernel(
    A_x: jax.Array,
    A_Lambda_re: jax.Array,
    A_Lambda_im: jax.Array,
    A_B_re: jax.Array,
    A_B_im: jax.Array,
    A_C_re: jax.Array,
    A_C_im: jax.Array,
    A_log_dt: jax.Array,
    A_Dskip: jax.Array,
    B_x: jax.Array,
    B_w_gate: jax.Array,
    B_w_up: jax.Array,
    B_w_down: jax.Array,
):
    return _impl(A_x, A_Lambda_re, A_Lambda_im, A_B_re, A_B_im, A_C_re, A_C_im, A_log_dt, A_Dskip, B_x, B_w_gate, B_w_up, B_w_down)
```

```python
import functools

import jax
import jax.numpy as jnp
import numpy as np
from jax import lax
import jax.experimental.pallas as pl
import jax.experimental.pallas.tpu as pltpu

BF = jnp.bfloat16
F32 = jnp.float32
U32 = jnp.uint32

LANE = 128
R = 256
S = 8
TS = 8 * S
XPAD = 16
OPAD = 8
GELU_C0 = float(np.sqrt(2.0 / np.pi))
GELU_C1 = float(np.sqrt(2.0 / np.pi) * 0.044715)


def _cmul(ar, ai, br, bi):
    return ar * br - ai * bi, ar * bi + ai * br


def _nt_dot(a, b):
    return lax.dot_general(a, b, (((1,), (1,)), ((), ())), preferred_element_type=F32)


def _nn_dot(a, b):
    return jnp.dot(a, b, preferred_element_type=F32)


def _pack(v):
    return pltpu.bitcast(v.astype(BF), U32)


def _unpack(v):
    return pltpu.bitcast(v, BF)


class _Background:
    def __init__(self):
        self.queue = []

    def add(self, gen):
        self.queue.append(gen)

    def step(self, n):
        while n > 0 and self.queue:
            if next(self.queue[0], "done") == "done":
                self.queue.pop(0)
            else:
                n -= 1

    def drain(self):
        self.step(1 << 30)


def _x_groups(L):
    rest = L - 2 * R
    return (R, R, rest // 2, rest - rest // 2)


def _make_kernel(L, D, P, F):
    NC = D // LANE
    NR = L // R
    xg = _x_groups(L)
    xoff = [int(v) for v in np.cumsum((0,) + xg)]
    fch = [(f0, min(LANE, F - f0)) for f0 in range(0, F, LANE)]
    bch = list(range(P // LANE))
    order = ("x0", "b0", "b1", "x1", "bim", "vec", "x2", "x3", "gu", "dc")

    def kernel(x_hbm, lre_hbm, lim_hbm, ldt_hbm, bre_hbm, bim_hbm, cre_hbm, cim_hbm, dsk_hbm,
               wg_hbm, wu_hbm, wd_hbm, o_hbm, *scratch):
        scratch = list(scratch)
        xbufs = [scratch.pop(0) for _ in xg]
        obufs = [scratch.pop(0) for _ in range(NR)]
        (v_lre, v_lim, v_ldt, v_dsk, bre0, bre1, bim, cre, cim, cpr, cpi, wg, wu, wd,
         xp, res, ubuf, hbuf, act, tab, sem) = scratch

        def col_groups(src, dst, s, r0, r1):
            return [pltpu.make_async_copy(src.at[pl.ds(r0, r1 - r0), pl.ds(c * LANE, LANE)],
                                          dst.at[c, pl.ds(0, r1 - r0), :], sem.at[s])
                    for c in range(NC)]

        def whole(pairs, s):
            return [pltpu.make_async_copy(a, b, sem.at[s]) for a, b in pairs]

        defs = {
            "b0": lambda s: col_groups(bre_hbm, bre0, s, 0, P // 2),
            "b1": lambda s: col_groups(bre_hbm, bre1, s, P // 2, P),
            "bim": lambda s: col_groups(bim_hbm, bim, s, 0, P),
            "vec": lambda s: whole(((lre_hbm, v_lre), (lim_hbm, v_lim), (ldt_hbm, v_ldt), (dsk_hbm, v_dsk)), s),
            "gu": lambda s: col_groups(wg_hbm, wg, s, 0, F) + col_groups(wu_hbm, wu, s, 0, F),
            "dc": lambda s: whole(((cre_hbm, cre), (cim_hbm, cim)), s) + col_groups(wd_hbm, wd, s, 0, F),
        }
        for i in range(len(xg)):
            defs["x%d" % i] = functools.partial(col_groups, x_hbm, xbufs[i], r0=xoff[i], r1=xoff[i + 1])
        group = {}
        for s, name in enumerate(order):
            group[name] = defs[name](s=s) if name[0] == "x" else defs[name](s)
            for cp in group[name]:
                cp.start()
        osem = sem.at[len(order)]

        def wait(*names):
            for name in names:
                for cp in group[name]:
                    cp.wait()

        def ldw(ref, r0, rn, cs=tuple(range(NC))):
            u = ref.bitcast(U32)
            return _unpack(jnp.concatenate([u[c, r0 // 2:(r0 + rn) // 2, :] for c in cs], axis=1))

        def ld(ref, r0, rn, c0=None, cn=None):
            if c0 is None:
                return _unpack(ref[r0 // 2:(r0 + rn) // 2, :])
            return _unpack(ref[r0 // 2:(r0 + rn) // 2, c0:c0 + cn])

        def ln_pieces(t_lo, t_hi):
            for t0 in range(t_lo, t_hi, TS):
                gi = max(i for i in range(len(xg)) if xoff[i] <= t0)
                xu = xbufs[gi].bitcast(U32)
                q0 = (t0 - xoff[gi]) // 2
                rows = []
                for ip in range(S // 2):
                    w = jnp.concatenate(
                        [xu[c, pl.ds(q0 + ip, 8, stride=S // 2), :] for c in range(NC)], axis=1)
                    rows.append(pltpu.bitcast(w << 16, F32))
                    rows.append(pltpu.bitcast(w & np.uint32(0xFFFF0000), F32))
                x = jnp.concatenate(rows, axis=0)
                res[t0:t0 + TS, :] = x
                m = jnp.mean(x, axis=-1, keepdims=True)
                yield
                xc = x - m
                v = jnp.mean(xc * xc, axis=-1, keepdims=True)
                yield
                xp[t0 // 2:(t0 + TS) // 2, :] = _pack(xc * lax.rsqrt(v + 1e-5))
                yield

        def table_pieces():
            lre = v_lre[...].astype(F32).reshape(1, P)
            lim = v_lim[...].astype(F32).reshape(1, P)
            dt = jnp.exp(v_ldt[...].astype(F32).reshape(1, P)).astype(BF).astype(F32)
            zr, zi = dt * lre, dt * lim
            yield
            mag = jnp.exp(zr)
            ar = mag * jnp.cos(zi)
            yield
            ai = mag * jnp.sin(zi)
            yield
            nr, ni = ar - 1.0, ai
            big = jnp.abs(lre) >= jnp.abs(lim)
            ratio = jnp.where(big, lim, lre) / jnp.where(big, lre, lim)
            den = jnp.where(big, lre + lim * ratio, lre * ratio + lim)
            sr = jnp.where(big, nr + ni * ratio, nr * ratio + ni) / den
            si = jnp.where(big, ni - nr * ratio, ni * ratio - nr) / den
            sub = lax.broadcasted_iota(jnp.int32, (8, P), 0)
            tab[0] = jnp.broadcast_to(ar, (8, P))
            tab[1] = jnp.broadcast_to(ai, (8, P))
            tab[8] = jnp.broadcast_to(2.0 * sr, (8, P))
            tab[9] = jnp.broadcast_to(2.0 * si, (8, P))
            yield
            pr, pi = ar, ai
            n = 1
            while n < S:
                pr, pi = _cmul(pr, pi, pr, pi)
                n *= 2
            for k, d in enumerate((1, 2, 4)):
                tab[2 + 2 * k] = jnp.where(sub >= d, jnp.broadcast_to(pr, (8, P)), 0.0)
                tab[3 + 2 * k] = jnp.where(sub >= d, jnp.broadcast_to(pi, (8, P)), 0.0)
                pr, pi = _cmul(pr, pi, pr, pi)
            yield

        def c_pieces(nparts):
            for part in range(nparts):
                r0, r1 = part * D // nparts, (part + 1) * D // nparts
                sr2, si2 = tab[8][0:1, :], tab[9][0:1, :]
                c_re = cre[r0:r1, :].astype(F32)
                c_im = cim[r0:r1, :].astype(F32)
                cpr[r0 // 2:r1 // 2, :] = _pack(c_re * sr2 - c_im * si2)
                cpi[r0 // 2:r1 // 2, :] = _pack(-(c_re * si2) - c_im * sr2)
                yield

        def scan_pieces():
            sub = lax.broadcasted_iota(jnp.int32, (8, P), 0)
            cr = ci = jnp.zeros((8, P), F32)
            for base in range(0, L, TS):
                ar, ai = tab[0], tab[1]
                fr = ubuf[base:base + 8, 0:P]
                fi = ubuf[base:base + 8, P:2 * P]
                for i in range(1, S):
                    ur = ubuf[base + 8 * i:base + 8 * i + 8, 0:P]
                    ui = ubuf[base + 8 * i:base + 8 * i + 8, P:2 * P]
                    fr, fi = ar * fr - ai * fi + ur, ar * fi + ai * fr + ui
                    if i == S // 2 - 1:
                        yield
                yield
                hr = jnp.where(sub == 0, cr, pltpu.roll(fr, 1, 0))
                hi = jnp.where(sub == 0, ci, pltpu.roll(fi, 1, 0))
                for k, d in enumerate((1, 2, 4)):
                    qr, qi = pltpu.roll(hr, d, 0), pltpu.roll(hi, d, 0)
                    tr, ti = tab[2 + 2 * k], tab[3 + 2 * k]
                    hr, hi = hr + (tr * qr - ti * qi), hi + (tr * qi + ti * qr)
                yield
                for i in range(S):
                    ur = ubuf[base + 8 * i:base + 8 * i + 8, 0:P]
                    ui = ubuf[base + 8 * i:base + 8 * i + 8, P:2 * P]
                    pr, pi = hr, hi
                    hr, hi = ar * hr - ai * hi + ur, ar * hi + ai * hr + ui
                    if i % 2 == 1:
                        q = (base + 8 * (i - 1)) // 2
                        hbuf[q:q + 8, 0:P] = _pack(jnp.concatenate([pr, hr], axis=0))
                        hbuf[q:q + 8, P:2 * P] = _pack(jnp.concatenate([pi, hi], axis=0))
                    if i == S // 2 - 1:
                        yield
                cr = jnp.broadcast_to(hr[7:8, :], (8, P))
                ci = jnp.broadcast_to(hi[7:8, :], (8, P))
                yield

        bg = _Background()
        ln_per_tile = 3 * (R // TS)

        def b_jobs(r0, rn, part, chunks, pieces=0):
            for c in chunks:
                if part == 1:
                    w = ldw(bim, c * LANE, LANE)
                elif c < len(bch) // 2:
                    w = ldw(bre0, c * LANE, LANE)
                else:
                    w = ldw(bre1, c * LANE - P // 2, LANE)
                col = part * P + c * LANE
                ubuf[r0:r0 + rn, col:col + LANE] = _nt_dot(ld(xp, r0, rn), w)
                bg.step(pieces)

        half = len(bch) // 2
        wait("x0")
        bg.add(ln_pieces(0, R))
        bg.drain()
        wait("b0")
        b_jobs(0, R, 0, bch[:half])
        wait("b1")
        b_jobs(0, R, 0, bch[half:])
        wait("x1")
        bg.add(ln_pieces(R, 2 * R))
        bg.step(ln_per_tile // 2)
        b_jobs(R, R // 2, 0, bch, pieces=2)
        bg.drain()
        b_jobs(R + R // 2, R // 2, 0, bch)
        wait("bim", "vec")
        bg.add(table_pieces())
        b_jobs(0, R, 1, bch, pieces=2)
        bg.drain()
        b_jobs(R, R, 1, bch[:1])
        wait("x2")
        bg.add(ln_pieces(2 * R, 3 * R))
        b_jobs(R, R, 1, bch[1:], pieces=5)
        bg.drain()
        for r in range(2, NR):
            jobs = [(part, c) for part in range(2) for c in bch]
            first = 0
            if r + 1 < NR:
                if (r + 1) * R == xoff[3]:
                    b_jobs(r * R, R, 0, bch[:1])
                    first = 1
                    wait("x3")
                bg.add(ln_pieces((r + 1) * R, (r + 2) * R))
            for part, c in jobs[first:]:
                b_jobs(r * R, R, part, [c], pieces=2)
            bg.drain()
        wait("gu")

        scan = scan_pieces()
        n_scan = (L // TS) * 5
        n_jobs = NR * 2 * len(fch)
        state = {"jobs": 0, "scan": 0}

        def tick():
            state["jobs"] += 1
            want = min(n_scan, -(-n_scan * state["jobs"] * 10 // (n_jobs * 9)))
            while state["scan"] < want:
                next(scan)
                state["scan"] += 1

        for r in range(NR):
            for f0, fn in fch:
                g = _nt_dot(ld(xp, r * R, R), ldw(wg, f0, fn))
                tick()
                u = _nt_dot(ld(xp, r * R, R), ldw(wu, f0, fn))
                last = r == NR - 1 and f0 == fch[-1][0]
                if last:
                    for _ in scan:
                        pass
                    wait("dc")
                t = jnp.tanh(g * (GELU_C0 + GELU_C1 * (g * g)))
                act[r * R // 2:(r + 1) * R // 2, f0:f0 + fn] = _pack((g * u) * (0.5 + 0.5 * t))
                if not last:
                    tick()

        bg.add(c_pieces(8))
        dsk = v_dsk[...].astype(F32).reshape(1, D)
        out_copies = []
        for r in range(NR):
            rows = slice(r * R, (r + 1) * R)
            down = []
            if r == 0:
                for c in range(NC):
                    down.append(_nn_dot(ld(act, r * R, R), ldw(wd, 0, F, (c,))))
                    bg.step(2)
                bg.drain()
            nsplit = R // TS if r == NR - 1 else 1
            for c in range(NC):
                cols = slice(c * LANE, (c + 1) * LANE)
                y = res[rows, cols] + ld(xp, r * R, R, c * LANE, LANE).astype(F32) * dsk[:, cols]
                y = y + (down[c] if r == 0 else _nn_dot(ld(act, r * R, R), ldw(wd, 0, F, (c,))))
                y = y + _nt_dot(ld(hbuf, r * R, R, 0, P), ld(cpr, c * LANE, LANE))
                y = y + _nt_dot(ld(hbuf, r * R, R, P, P), ld(cpi, c * LANE, LANE))
                for n in range(R // TS):
                    for i in range(S):
                        obufs[r][c, pl.ds(n * TS + i, 8, stride=S), :] = y[n * TS + 8 * i:n * TS + 8 * i + 8, :]
                    if (n + 1) % (R // TS // nsplit) == 0:
                        a = (n + 1) * TS - R // nsplit
                        cp = pltpu.make_async_copy(
                            obufs[r].at[c, pl.ds(a, R // nsplit), :],
                            o_hbm.at[pl.ds(r * R + a, R // nsplit), pl.ds(c * LANE, LANE)], osem)
                        cp.start()
                        out_copies.append(cp)
        for cp in out_copies:
            cp.wait()

    scratch_shapes = (
        [pltpu.VMEM((NC, n + XPAD, LANE), BF) for n in xg]
        + [pltpu.VMEM((NC, R + OPAD, LANE), F32) for _ in range(NR)]
        + [pltpu.VMEM((P,), BF)] * 3 + [pltpu.VMEM((D,), BF)]
        + [pltpu.VMEM((NC, P // 2, LANE), BF)] * 2 + [pltpu.VMEM((NC, P, LANE), BF)]
        + [pltpu.VMEM((D, P), BF)] * 2
        + [pltpu.VMEM((D // 2, P), U32)] * 2
        + [pltpu.VMEM((NC, F, LANE), BF)] * 3
        + [pltpu.VMEM((L // 2, D), U32),
           pltpu.VMEM((L, D), F32),
           pltpu.VMEM((L, 2 * P), F32),
           pltpu.VMEM((L // 2, 2 * P), U32),
           pltpu.VMEM((L // 2, F), U32),
           pltpu.VMEM((10, 8, P), F32),
           pltpu.SemaphoreType.DMA((len(order) + 1,))])
    return kernel, scratch_shapes


@jax.jit
def pallas_parallel_sum__ssm_conv_s5__geglu_ffn__prompt_kernel(
    A_x: jax.Array,
    A_Lambda_re: jax.Array,
    A_Lambda_im: jax.Array,
    A_B_re: jax.Array,
    A_B_im: jax.Array,
    A_C_re: jax.Array,
    A_C_im: jax.Array,
    A_log_dt: jax.Array,
    A_Dskip: jax.Array,
    B_x: jax.Array,
    B_w_gate: jax.Array,
    B_w_up: jax.Array,
    B_w_down: jax.Array,
):
    del B_x
    Bsz, L, D = A_x.shape
    P = A_B_re.shape[0]
    F = B_w_gate.shape[1]
    assert Bsz == 1 and L % (4 * R) == 0 and D % LANE == 0 and P % (2 * LANE) == 0 and F % 16 == 0
    kernel, scratch_shapes = _make_kernel(L, D, P, F)
    hbm = pl.BlockSpec(memory_space=pltpu.HBM)
    out = pl.pallas_call(
        kernel,
        in_specs=[hbm] * 12,
        out_specs=hbm,
        out_shape=jax.ShapeDtypeStruct((L, D), F32),
        scratch_shapes=scratch_shapes,
        compiler_params=pltpu.CompilerParams(
            vmem_limit_bytes=100 * 2**20, disable_semaphore_checks=True),
    )(A_x.reshape(L, D), A_Lambda_re, A_Lambda_im, A_log_dt, A_B_re, A_B_im, A_C_re, A_C_im, A_Dskip,
      B_w_gate.T, B_w_up.T, B_w_down)
    return out.reshape(1, L, D)
```

```python
import functools

import jax
import jax.numpy as jnp
import numpy as np
from jax import lax
import jax.experimental.pallas as pl
import jax.experimental.pallas.tpu as pltpu

BF = jnp.bfloat16
F32 = jnp.float32
U32 = jnp.uint32

LANE = 128
R = 256
S = 8
TS = 8 * S
GELU_C0 = float(np.sqrt(2.0 / np.pi))
GELU_C1 = float(np.sqrt(2.0 / np.pi) * 0.044715)


def _cmul(ar, ai, br, bi):
    return ar * br - ai * bi, ar * bi + ai * br


def _nt_dot(a, b):
    return lax.dot_general(a, b, (((1,), (1,)), ((), ())), preferred_element_type=F32)


def _nn_dot(a, b):
    return jnp.dot(a, b, preferred_element_type=F32)


def _pack(v):
    return pltpu.bitcast(v.astype(BF), U32)


def _unpack(v):
    return pltpu.bitcast(v, BF)


class _Background:
    def __init__(self):
        self.queue = []

    def add(self, gen):
        self.queue.append(gen)

    def step(self, n):
        while n > 0 and self.queue:
            if next(self.queue[0], "done") == "done":
                self.queue.pop(0)
            else:
                n -= 1

    def drain(self):
        self.step(1 << 30)


def _x_groups(L):
    rest = L - 2 * R
    return (R, R, rest // 2, rest - rest // 2)


def _make_kernel(L, D, P, F):
    NC = D // LANE
    NR = L // R
    xg = _x_groups(L)
    xoff = [int(v) for v in np.cumsum((0,) + xg)]
    fch = [(f0, min(LANE, F - f0)) for f0 in range(0, F, LANE)]
    bch = list(range(P // LANE))
    order = ("x0", "b0", "b1", "x1", "bim", "vec", "x2", "x3", "gu", "dc")

    def kernel(x_hbm, lre_hbm, lim_hbm, ldt_hbm, bre_hbm, bim_hbm, cre_hbm, cim_hbm, dsk_hbm,
               wg_hbm, wu_hbm, wd_hbm, o_hbm, *scratch):
        scratch = list(scratch)
        xbufs = [scratch.pop(0) for _ in xg]
        obufs = [scratch.pop(0) for _ in range(NR)]
        (v_lre, v_lim, v_ldt, v_dsk, bre0, bre1, bim, cre, cim, cpr, cpi, wg, wu, wd,
         xp, res, ubuf, hbuf, act, tab, sem) = scratch

        def col_groups(src, dst, s, r0, r1):
            return [pltpu.make_async_copy(src.at[pl.ds(r0, r1 - r0), pl.ds(c * LANE, LANE)],
                                          dst.at[c, pl.ds(0, r1 - r0), :], sem.at[s])
                    for c in range(NC)]

        def whole(pairs, s):
            return [pltpu.make_async_copy(a, b, sem.at[s]) for a, b in pairs]

        defs = {
            "b0": lambda s: col_groups(bre_hbm, bre0, s, 0, P // 2),
            "b1": lambda s: col_groups(bre_hbm, bre1, s, P // 2, P),
            "bim": lambda s: col_groups(bim_hbm, bim, s, 0, P),
            "vec": lambda s: whole(((lre_hbm, v_lre), (lim_hbm, v_lim), (ldt_hbm, v_ldt), (dsk_hbm, v_dsk)), s),
            "gu": lambda s: col_groups(wg_hbm, wg, s, 0, F) + col_groups(wu_hbm, wu, s, 0, F),
            "dc": lambda s: whole(((cre_hbm, cre), (cim_hbm, cim)), s) + col_groups(wd_hbm, wd, s, 0, F),
        }
        for i in range(len(xg)):
            defs["x%d" % i] = functools.partial(col_groups, x_hbm.bitcast(U32), xbufs[i], r0=xoff[i] // 2, r1=xoff[i + 1] // 2)
        group = {}
        for s, name in enumerate(order):
            group[name] = defs[name](s=s) if name[0] == "x" else defs[name](s)
            for cp in group[name]:
                cp.start()
        osem = sem.at[len(order)]

        def wait(*names):
            for name in names:
                for cp in group[name]:
                    cp.wait()

        def ldw(ref, r0, rn, cs=tuple(range(NC))):
            return jnp.concatenate([ref[c, r0:r0 + rn, :] for c in cs], axis=1)

        def ld(ref, r0, rn, c0=None, cn=None):
            if c0 is None:
                return _unpack(ref[r0 // 2:(r0 + rn) // 2, :])
            return _unpack(ref[r0 // 2:(r0 + rn) // 2, c0:c0 + cn])

        def ln_pieces(t_lo, t_hi):
            for t0 in range(t_lo, t_hi, TS):
                gi = max(i for i in range(len(xg)) if xoff[i] <= t0)
                xu = xbufs[gi]
                q0 = (t0 - xoff[gi]) // 2
                rows = []
                for ip in range(S // 2):
                    w = jnp.concatenate(
                        [xu[c, pl.ds(q0 + ip, 8, stride=S // 2), :] for c in range(NC)], axis=1)
                    rows.append(pltpu.bitcast(w << 16, F32))
                    rows.append(pltpu.bitcast(w & np.uint32(0xFFFF0000), F32))
                x = jnp.concatenate(rows, axis=0)
                res[t0:t0 + TS, :] = x
                m = jnp.mean(x, axis=-1, keepdims=True)
                yield
                xc = x - m
                v = jnp.mean(xc * xc, axis=-1, keepdims=True)
                yield
                xp[t0 // 2:(t0 + TS) // 2, :] = _pack(xc * lax.rsqrt(v + 1e-5))
                yield

        def table_pieces():
            lre = v_lre[...].astype(F32).reshape(1, P)
            lim = v_lim[...].astype(F32).reshape(1, P)
            dt = jnp.exp(v_ldt[...].astype(F32).reshape(1, P)).astype(BF).astype(F32)
            zr, zi = dt * lre, dt * lim
            yield
            mag = jnp.exp(zr)
            ar = mag * jnp.cos(zi)
            yield
            ai = mag * jnp.sin(zi)
            yield
            nr, ni = ar - 1.0, ai
            big = jnp.abs(lre) >= jnp.abs(lim)
            ratio = jnp.where(big, lim, lre) / jnp.where(big, lre, lim)
            den = jnp.where(big, lre + lim * ratio, lre * ratio + lim)
            sr = jnp.where(big, nr + ni * ratio, nr * ratio + ni) / den
            si = jnp.where(big, ni - nr * ratio, ni * ratio - nr) / den
            sub = lax.broadcasted_iota(jnp.int32, (8, P), 0)
            tab[0] = jnp.broadcast_to(ar, (8, P))
            tab[1] = jnp.broadcast_to(ai, (8, P))
            tab[8] = jnp.broadcast_to(2.0 * sr, (8, P))
            tab[9] = jnp.broadcast_to(2.0 * si, (8, P))
            yield
            pr, pi = ar, ai
            n = 1
            while n < S:
                pr, pi = _cmul(pr, pi, pr, pi)
                n *= 2
            for k, d in enumerate((1, 2, 4)):
                tab[2 + 2 * k] = jnp.where(sub >= d, jnp.broadcast_to(pr, (8, P)), 0.0)
                tab[3 + 2 * k] = jnp.where(sub >= d, jnp.broadcast_to(pi, (8, P)), 0.0)
                pr, pi = _cmul(pr, pi, pr, pi)
            yield

        def c_pieces(nparts):
            for part in range(nparts):
                r0, r1 = part * D // nparts, (part + 1) * D // nparts
                sr2, si2 = tab[8][0:1, :], tab[9][0:1, :]
                c_re = cre[r0:r1, :].astype(F32)
                c_im = cim[r0:r1, :].astype(F32)
                cpr[r0 // 2:r1 // 2, :] = _pack(c_re * sr2 - c_im * si2)
                cpi[r0 // 2:r1 // 2, :] = _pack(-(c_re * si2) - c_im * sr2)
                yield

        def scan_pieces():
            sub = lax.broadcasted_iota(jnp.int32, (8, P), 0)
            cr = ci = jnp.zeros((8, P), F32)
            for base in range(0, L, TS):
                ar, ai = tab[0], tab[1]
                fr = ubuf[base:base + 8, 0:P]
                fi = ubuf[base:base + 8, P:2 * P]
                for i in range(1, S):
                    ur = ubuf[base + 8 * i:base + 8 * i + 8, 0:P]
                    ui = ubuf[base + 8 * i:base + 8 * i + 8, P:2 * P]
                    fr, fi = ar * fr - ai * fi + ur, ar * fi + ai * fr + ui
                    if i == S // 2 - 1:
                        yield
                yield
                hr = jnp.where(sub == 0, cr, pltpu.roll(fr, 1, 0))
                hi = jnp.where(sub == 0, ci, pltpu.roll(fi, 1, 0))
                for k, d in enumerate((1, 2, 4)):
                    qr, qi = pltpu.roll(hr, d, 0), pltpu.roll(hi, d, 0)
                    tr, ti = tab[2 + 2 * k], tab[3 + 2 * k]
                    hr, hi = hr + (tr * qr - ti * qi), hi + (tr * qi + ti * qr)
                yield
                for i in range(S):
                    ur = ubuf[base + 8 * i:base + 8 * i + 8, 0:P]
                    ui = ubuf[base + 8 * i:base + 8 * i + 8, P:2 * P]
                    pr, pi = hr, hi
                    hr, hi = ar * hr - ai * hi + ur, ar * hi + ai * hr + ui
                    if i % 2 == 1:
                        q = (base + 8 * (i - 1)) // 2
                        hbuf[q:q + 8, 0:P] = _pack(jnp.concatenate([pr, hr], axis=0))
                        hbuf[q:q + 8, P:2 * P] = _pack(jnp.concatenate([pi, hi], axis=0))
                    if i == S // 2 - 1:
                        yield
                cr = jnp.broadcast_to(hr[7:8, :], (8, P))
                ci = jnp.broadcast_to(hi[7:8, :], (8, P))
                yield

        bg = _Background()
        ln_per_tile = 3 * (R // TS)

        def b_jobs(r0, rn, part, chunks, pieces=0):
            for c in chunks:
                if part == 1:
                    w = ldw(bim, c * LANE, LANE)
                elif c < len(bch) // 2:
                    w = ldw(bre0, c * LANE, LANE)
                else:
                    w = ldw(bre1, c * LANE - P // 2, LANE)
                col = part * P + c * LANE
                ubuf[r0:r0 + rn, col:col + LANE] = _nt_dot(ld(xp, r0, rn), w)
                bg.step(pieces)

        half = len(bch) // 2
        wait("x0")
        bg.add(ln_pieces(0, R))
        bg.drain()
        wait("b0")
        b_jobs(0, R, 0, bch[:half])
        wait("b1")
        b_jobs(0, R, 0, bch[half:])
        wait("x1")
        bg.add(ln_pieces(R, 2 * R))
        bg.step(ln_per_tile // 2)
        b_jobs(R, R // 2, 0, bch, pieces=2)
        bg.drain()
        b_jobs(R + R // 2, R // 2, 0, bch)
        wait("bim", "vec")
        bg.add(table_pieces())
        b_jobs(0, R, 1, bch, pieces=2)
        bg.drain()
        b_jobs(R, R, 1, bch[:1])
        wait("x2")
        bg.add(ln_pieces(2 * R, 3 * R))
        b_jobs(R, R, 1, bch[1:], pieces=5)
        bg.drain()
        for r in range(2, NR):
            jobs = [(part, c) for part in range(2) for c in bch]
            first = 0
            if r + 1 < NR:
                if (r + 1) * R == xoff[3]:
                    b_jobs(r * R, R, 0, bch[:1])
                    first = 1
                    wait("x3")
                bg.add(ln_pieces((r + 1) * R, (r + 2) * R))
            for part, c in jobs[first:]:
                b_jobs(r * R, R, part, [c], pieces=2)
            bg.drain()
        wait("gu")

        scan = scan_pieces()
        n_scan = (L // TS) * 5
        n_jobs = NR * 2 * len(fch)
        state = {"jobs": 0, "scan": 0}

        def tick():
            state["jobs"] += 1
            want = min(n_scan, -(-n_scan * state["jobs"] * 10 // (n_jobs * 9)))
            while state["scan"] < want:
                next(scan)
                state["scan"] += 1

        for r in range(NR):
            for f0, fn in fch:
                g = _nt_dot(ld(xp, r * R, R), ldw(wg, f0, fn))
                tick()
                u = _nt_dot(ld(xp, r * R, R), ldw(wu, f0, fn))
                last = r == NR - 1 and f0 == fch[-1][0]
                if last:
                    for _ in scan:
                        pass
                    wait("dc")
                t = jnp.tanh(g * (GELU_C0 + GELU_C1 * (g * g)))
                act[r * R // 2:(r + 1) * R // 2, f0:f0 + fn] = _pack((g * u) * (0.5 + 0.5 * t))
                if not last:
                    tick()

        bg.add(c_pieces(8))
        dsk = v_dsk[...].astype(F32).reshape(1, D)
        out_copies = []
        for r in range(NR):
            rows = slice(r * R, (r + 1) * R)
            down = []
            if r == 0:
                for c in range(NC):
                    down.append(_nn_dot(ld(act, r * R, R), ldw(wd, 0, F, (c,))))
                    bg.step(2)
                bg.drain()
            nsplit = R // TS if r == NR - 1 else 1
            for c in range(NC):
                cols = slice(c * LANE, (c + 1) * LANE)
                y = res[rows, cols] + ld(xp, r * R, R, c * LANE, LANE).astype(F32) * dsk[:, cols]
                y = y + (down[c] if r == 0 else _nn_dot(ld(act, r * R, R), ldw(wd, 0, F, (c,))))
                y = y + _nt_dot(ld(hbuf, r * R, R, 0, P), ld(cpr, c * LANE, LANE))
                y = y + _nt_dot(ld(hbuf, r * R, R, P, P), ld(cpi, c * LANE, LANE))
                for n in range(R // TS):
                    for i in range(S):
                        obufs[r][c, pl.ds(n * TS + i, 8, stride=S), :] = y[n * TS + 8 * i:n * TS + 8 * i + 8, :]
                    if (n + 1) % (R // TS // nsplit) == 0:
                        a = (n + 1) * TS - R // nsplit
                        cp = pltpu.make_async_copy(
                            obufs[r].at[c, pl.ds(a, R // nsplit), :],
                            o_hbm.at[pl.ds(r * R + a, R // nsplit), pl.ds(c * LANE, LANE)], osem)
                        cp.start()
                        out_copies.append(cp)
        for cp in out_copies:
            cp.wait()

    scratch_shapes = (
        [pltpu.VMEM((NC, n // 2, LANE), U32) for n in xg]
        + [pltpu.VMEM((NC, R, LANE), F32) for _ in range(NR)]
        + [pltpu.VMEM((P,), BF)] * 3 + [pltpu.VMEM((D,), BF)]
        + [pltpu.VMEM((NC, P // 2, LANE), BF)] * 2 + [pltpu.VMEM((NC, P, LANE), BF)]
        + [pltpu.VMEM((D, P), BF)] * 2
        + [pltpu.VMEM((D // 2, P), U32)] * 2
        + [pltpu.VMEM((NC, F, LANE), BF)] * 3
        + [pltpu.VMEM((L // 2, D), U32),
           pltpu.VMEM((L, D), F32),
           pltpu.VMEM((L, 2 * P), F32),
           pltpu.VMEM((L // 2, 2 * P), U32),
           pltpu.VMEM((L // 2, F), U32),
           pltpu.VMEM((10, 8, P), F32),
           pltpu.SemaphoreType.DMA((len(order) + 1,))])
    return kernel, scratch_shapes


@jax.jit
def pallas_parallel_sum__ssm_conv_s5__geglu_ffn__prompt_kernel(
    A_x: jax.Array,
    A_Lambda_re: jax.Array,
    A_Lambda_im: jax.Array,
    A_B_re: jax.Array,
    A_B_im: jax.Array,
    A_C_re: jax.Array,
    A_C_im: jax.Array,
    A_log_dt: jax.Array,
    A_Dskip: jax.Array,
    B_x: jax.Array,
    B_w_gate: jax.Array,
    B_w_up: jax.Array,
    B_w_down: jax.Array,
):
    del B_x
    Bsz, L, D = A_x.shape
    P = A_B_re.shape[0]
    F = B_w_gate.shape[1]
    assert Bsz == 1 and L % (4 * R) == 0 and D % LANE == 0 and P % (2 * LANE) == 0 and F % 16 == 0
    kernel, scratch_shapes = _make_kernel(L, D, P, F)
    hbm = pl.BlockSpec(memory_space=pltpu.HBM)
    out = pl.pallas_call(
        kernel,
        in_specs=[hbm] * 12,
        out_specs=hbm,
        out_shape=jax.ShapeDtypeStruct((L, D), F32),
        scratch_shapes=scratch_shapes,
        compiler_params=pltpu.CompilerParams(
            vmem_limit_bytes=100 * 2**20, disable_semaphore_checks=True),
    )(A_x.reshape(L, D), A_Lambda_re, A_Lambda_im, A_log_dt, A_B_re, A_B_im, A_C_re, A_C_im, A_Dskip,
      B_w_gate.T, B_w_up.T, B_w_down)
    return out.reshape(1, L, D)
```
